```python
import os as _os
_os.environ.setdefault("JAX_PLATFORMS", "cpu")
import jax
import jax.numpy as jnp

def _softmax(x, axis=-1):
    return jax.nn.softmax(x, axis=axis)
def _gelu(x):
    return jax.nn.gelu(x, approximate=True)
def _silu(x):
    return jax.nn.silu(x)
def _sigmoid(x):
    return jax.nn.sigmoid(x)
def _layernorm(x, axis=-1, eps=1e-5):
    m = jnp.mean(x, axis=axis, keepdims=True)
    v = jnp.var(x, axis=axis, keepdims=True)
    return (x - m) / jnp.sqrt(v + eps)
def _scatter_add(tgt, idx, src, axis=0):
    return tgt.at[idx].add(src)
def _segment_sum(src, seg, n):
    return jax.ops.segment_sum(src, seg, n)
class _Rng:
    def __init__(self, key):
        self._k = key
    def _next(self):
        self._k, sub = jax.random.split(self._k)
        return sub
    def normal(self, shape):
        return jax.random.normal(self._next(), shape, dtype=jnp.bfloat16)
    def randint(self, lo, hi, shape):
        return jax.random.randint(self._next(), shape, lo, hi, dtype=jnp.int32)
    def uniform(self, shape, lo=0.0, hi=1.0):
        return jax.random.uniform(self._next(), shape, jnp.bfloat16, lo, hi)
    def permutation(self, n):
        return jax.random.permutation(self._next(), n)


kernel_name = 'gated_mix__sliding_block__sliding_local_dilated__prompt'

def setup_inputs():
    _rng = _Rng(jax.random.key(int.from_bytes(__import__("os").urandom(4), "little")))
    _w = (lambda a: (lambda t: t.astype(jnp.bfloat16) if jnp.issubdtype(t.dtype, jnp.floating) else t)(jnp.asarray(a)))
    def _A_setup():
        B, S, D = 1, 2048, 640
        return {
            "x": _w((lambda *s: _rng.normal(s) * 0.05)(B, S, D)),
            "wqkv": _w((lambda *s: _rng.normal(s) * 0.8)(D, 3 * D)),
            "wo": _w((lambda *s: _rng.normal(s) * 0.05)(D, D)),
        }
    _A_in = _A_setup()

    def _B_setup():
        B, S, D = 1, 2048, 640
        return {
            "x": _w((lambda *s: _rng.normal(s) * 0.05)(B, S, D)),
            "wqkv": _w((lambda *s: _rng.normal(s) * 0.8)(D, 3 * D)),
            "wo": _w((lambda *s: _rng.normal(s) * 0.05)(D, D)),
        }
    _B_in = _B_setup()

    return {
        "A_x": _A_in["x"],
        "A_wqkv": _A_in["wqkv"],
        "A_wo": _A_in["wo"],
        "B_x": _B_in["x"],
        "B_wqkv": _B_in["wqkv"],
        "B_wo": _B_in["wo"],
        "gate_w": _w((lambda *s: _rng.normal(s) * 0.05)(640) * 16.0),
    }

def reference(A_x, A_wqkv, A_wo, B_x, B_wqkv, B_wo, gate_w):
    def _A_ref(x, wqkv, wo):
        B, S, D = x.shape
        H = 32; Dh = D // H; W = 256
        qkv = (lambda x, *d: x.transpose(*d))((x @ wqkv).reshape(B, S, 3, H, Dh), 2, 0, 3, 1, 4)
        q, k, v = qkv[0], qkv[1], qkv[2]
        scores = jnp.einsum("bhqd,bhkd->bhqk", q, k) * (Dh ** -0.5)
        idx = jnp.arange(S)
        mask = (idx[:, None] - idx[None, :] >= 0) & (idx[:, None] - idx[None, :] < W)
        scores = jnp.where(mask[None, None], scores, -1e9)
        p = _softmax(scores, axis=-1)
        o = jnp.einsum("bhqk,bhkd->bhqd", p, v)
        return (lambda x, *d: x.transpose(*d))(o, 0, 2, 1, 3).reshape(B, S, D) @ wo

    def _B_ref(x, wqkv, wo):
        B, S, D = x.shape
        H = 32; Dh = D // H
        W, dil = 8, 2
        qkv = (lambda x, *d: x.transpose(*d))((x @ wqkv).reshape(B, S, 3, H, Dh), 2, 0, 3, 1, 4)
        q, k, v = qkv[0], qkv[1], qkv[2]
        scale = Dh ** -0.5
        pos = jnp.arange(S)
        off = jnp.arange(W) * dil
        idx = pos[:, None] - off[None, :]
        mask = idx >= 0
        idx_c = jnp.where(mask, idx, 0).reshape(-1)
        kg = k[:, :, idx_c, :].reshape(B, H, S, W, Dh)
        vg = v[:, :, idx_c, :].reshape(B, H, S, W, Dh)
        logits = jnp.einsum("bhsd,bhswd->bhsw", q, kg) * scale
        logits = jnp.where(mask[None, None, :, :], logits, -1e9)
        attn = _softmax(logits, axis=-1)
        o = jnp.einsum("bhsw,bhswd->bhsd", attn, vg)
        return (lambda x, *d: x.transpose(*d))(o, 0, 2, 1, 3).reshape(B, S, D) @ wo

    x = A_x
    g = _sigmoid((x * gate_w).sum(-1, keepdims=True))
    a = _A_ref(x, A_wqkv, A_wo)
    b = _B_ref(x, B_wqkv, B_wo)
    return g * a + (1 - g) * b
```

```python
import math

import jax
import jax.numpy as jnp
from jax import lax
import jax.experimental.pallas as pl
import jax.experimental.pallas.tpu as pltpu

S = 2048
D = 640
NT = D // 128
DH = 20
BS = 512
QB = 128
WIN = 256
NG = 16
PADB = 16
NS = 3
NP = 4
RB = 16
LOG2E = math.log2(math.e)
SCALE = DH ** -0.5
NEG = -1e9
BIGNEG = -(2.0 ** 30)

F32 = jnp.float32
BF16 = jnp.bfloat16


def _nn(a, b):
    return lax.dot_general(a, b, (((1,), (0,)), ((), ())), preferred_element_type=F32)


def _nt(a, b):
    return lax.dot_general(a, b, (((1,), (1,)), ((), ())), preferred_element_type=F32)


def _tt(a, b):
    return lax.dot_general(a, b, (((0,), (1,)), ((), ())), preferred_element_type=F32)


def _kernel(xa_ref, wa_ref, woa_ref, wb_ref, wob_ref, gw_ref, out_ref,
            kp_ref, vt_ref, wkp_ref, wbt_ref, wobp_ref, tmp_ref,
            qt_ref, qb_ref, kb_ref, vb_ref, g_ref, oc_ref, s_ref, p_ref):
    i = pl.program_id(0)

    @pl.when(i == 0)
    def _prep():
        lane = lax.broadcasted_iota(jnp.int32, (WIN, 768), 1)
        kp_ref[0:WIN, :] = jnp.where(lane % 128 == 127, 1.0, 0.0).astype(BF16)
        vt_ref[:, 0:WIN] = jnp.zeros((NG * 48, WIN), BF16)
        kb_ref[:, 0:PADB, :] = jnp.zeros((NT, PADB, 128), F32)
        vb_ref[:, 0:PADB, :] = jnp.zeros((NT, PADB, 128), F32)
        p_ref[...] = jnp.zeros((NP, 384, 384), BF16)
        lane128 = lax.broadcasted_iota(jnp.int32, (D, 128), 1)
        for c in range(6):
            lo = D + 120 * c
            blk = wa_ref[:, lo:lo + 128].astype(F32)
            nvalid = min(120, D - 120 * c)
            wkp_ref[:, c * 128:(c + 1) * 128] = jnp.where(lane128 < nvalid, blk, 0.0).astype(BF16)
        for n in range(15):
            t_ = wb_ref[:, n * 128:(n + 1) * 128].T.astype(F32)
            for t in range(NT):
                tmp_ref[t, n * 128:(n + 1) * 128, :] = t_[:, t * 128:(t + 1) * 128]
        for p in range(3):
            for t in range(NT):
                for d in range(DH):
                    wbt_ref[p * D + d * 32:p * D + (d + 1) * 32, t * 128:(t + 1) * 128] = (
                        tmp_ref[t, pl.ds(p * D + d, 32, stride=DH), :].astype(BF16))
        for t in range(NT):
            tmp_ref[t, 0:D, :] = wob_ref[:, t * 128:(t + 1) * 128].astype(F32)
        for t in range(NT):
            for d in range(DH):
                wobp_ref[d * 32:(d + 1) * 32, t * 128:(t + 1) * 128] = (
                    tmp_ref[t, pl.ds(d, 32, stride=DH), :].astype(BF16))

    row0 = pl.multiple_of(i * BS, BS)

    xa = xa_ref[...]
    qt_ref[...] = _tt(wa_ref[:, 0:D], xa) * (SCALE * LOG2E)
    vt = _tt(wa_ref[:, 2 * D:3 * D], xa)
    ones8 = jnp.ones((8, BS), F32)
    for g in range(NG):
        blk = jnp.concatenate([vt[40 * g:40 * g + 40], ones8], axis=0).astype(BF16)
        vt_ref[48 * g:48 * g + 48, pl.ds(WIN + row0, BS)] = blk
    kp_ref[pl.ds(WIN + row0, BS), :] = _nn(xa, wkp_ref[...]).astype(BF16)
    gl = jnp.sum(xa.astype(F32) * gw_ref[...].astype(F32), axis=-1, keepdims=True)
    g_ref[...] = jnp.broadcast_to(jax.nn.sigmoid(gl), (BS, 128))

    xb = xa
    qb_ref[...] = _nt(xb, wbt_ref[0:D, :]) * (SCALE * LOG2E)
    kb = _nt(xb, wbt_ref[D:2 * D, :])
    vb = _nt(xb, wbt_ref[2 * D:3 * D, :])
    for t in range(NT):
        kb_ref[t, pl.ds(PADB + row0, BS), :] = kb[:, t * 128:(t + 1) * 128]
        vb_ref[t, pl.ds(PADB + row0, BS), :] = vb[:, t * 128:(t + 1) * 128]

    r40 = lax.broadcasted_iota(jnp.int32, (40, 128), 0)
    l40 = lax.broadcasted_iota(jnp.int32, (40, 128), 1)
    m0 = (r40 < 20) & (l40 < 64)
    m1 = (r40 >= 20) & (l40 >= 64)
    h0row = r40 < 20
    lo64 = l40 < 64
    r8 = lax.broadcasted_iota(jnp.int32, (8, 128), 0)
    negrow = jnp.where(r8 == 7, BIGNEG, 0.0).astype(F32)

    def band_mask(nn):
        r64 = lax.broadcasted_iota(jnp.int32, (64, 128 * nn), 0)
        q64 = lax.broadcasted_iota(jnp.int32, (64, 128 * nn), 1) % 64
        return r64 > q64

    NB = BS // QB
    items = [(m, c, sub) for m in range(NB) for c in range(6) for sub in range(2)]
    mxs, outs = {}, {}

    def groups(c):
        return list(range(3 * c, min(3 * c + 3, NG)))

    def stage_a(n):
        m, c, sub = items[n]
        gs = groups(c)
        nn = len(gs)
        tiles = []
        for j, g in enumerate(gs):
            qt = qt_ref[40 * g:40 * g + 40, m * QB:(m + 1) * QB]
            rq = pltpu.roll(qt, 64, 1)
            if sub == 0:
                tq = jnp.where(m0, qt, jnp.where(m1, rq, 0.0))
            else:
                tq = jnp.where(m0, rq, jnp.where(m1, qt, 0.0))
            parts = []
            if j > 0:
                parts.append(jnp.zeros((40 * j, 128), F32))
            parts.append(tq)
            if j < 2:
                parts.append(jnp.zeros((80 - 40 * j, 128), F32))
            parts.append(negrow)
            tiles.append(jnp.concatenate(parts, axis=0).astype(BF16))
        rhs = jnp.concatenate(tiles, axis=1)
        kwin = kp_ref[pl.ds(row0 + m * QB + sub * 64, 320), c * 128:(c + 1) * 128]
        s = _nn(kwin, rhs)
        s = jnp.concatenate([jnp.where(band_mask(nn), s[0:64], s[256:320]), s[64:256]], axis=0)
        s_ref[n % NS, :, 0:128 * nn] = s
        mxs[n] = jnp.max(s, axis=0, keepdims=True)

    def stage_b(n):
        m, c, sub = items[n]
        nn = len(groups(c))
        p = jnp.exp2(s_ref[n % NS, :, 0:128 * nn] - mxs.pop(n))
        mk = band_mask(nn)
        b = sub * 64
        p_ref[n % NP, b:b + 64, 0:128 * nn] = jnp.where(mk, p[0:64], 0.0).astype(BF16)
        p_ref[n % NP, b + 64:b + 256, 0:128 * nn] = p[64:256].astype(BF16)
        p_ref[n % NP, b + 256:b + 320, 0:128 * nn] = jnp.where(mk, 0.0, p[0:64]).astype(BF16)

    def stage_c(n):
        m, c, sub = items[n]
        for j, g in enumerate(groups(c)):
            ot = _nn(vt_ref[48 * g:48 * g + 48, pl.ds(row0 + m * QB, 384)],
                     p_ref[n % NP, :, j * 128:(j + 1) * 128])
            outs[(g, sub)] = ot[0:40] * (1.0 / ot[40:41])
        if c == 5 and sub == 1:
            pieces = []
            for g in range(NG):
                o0, o1 = outs.pop((g, 0)), outs.pop((g, 1))
                a_ = jnp.where(h0row, o0, pltpu.roll(o0, 64, 1))
                b_ = jnp.where(h0row, pltpu.roll(o1, 64, 1), o1)
                pieces.append(jnp.where(lo64, a_, b_))
            oa = jnp.concatenate(pieces, axis=0).T
            gate = g_ref[m * QB:(m + 1) * QB, :]
            for t in range(NT):
                oc_ref[m * QB:(m + 1) * QB, t * 128:(t + 1) * 128] = (
                    oa[:, t * 128:(t + 1) * 128] * gate).astype(BF16)

    def branch_b(lr):
        q = [qb_ref[lr:lr + RB, t * 128:(t + 1) * 128] for t in range(NT)]
        logits = []
        for w in range(8):
            kr = PADB + row0 + lr - 2 * w
            acc = None
            for t in range(NT):
                pr = q[t] * kb_ref[t, pl.ds(kr, RB), :]
                acc = pr if acc is None else acc + pr
            acc = acc + pltpu.roll(acc, 64, 1)
            acc = acc + pltpu.roll(acc, 32, 1)
            if lr < 2 * w:
                pos = row0 + lr + lax.broadcasted_iota(jnp.int32, (RB, 128), 0)
                acc = jnp.where(pos >= 2 * w, acc, NEG)
            logits.append(acc)
        mx = logits[0]
        for w in range(1, 8):
            mx = jnp.maximum(mx, logits[w])
        es = [jnp.exp2(l - mx) for l in logits]
        den = es[0]
        for w in range(1, 8):
            den = den + es[w]
        fac = (1.0 - g_ref[lr:lr + RB, :]) / den
        for t in range(NT):
            acc = None
            for w in range(8):
                kr = PADB + row0 + lr - 2 * w
                pr = es[w] * vb_ref[t, pl.ds(kr, RB), :]
                acc = pr if acc is None else acc + pr
            oc_ref[lr:lr + RB, D + t * 128:D + (t + 1) * 128] = (acc * fac).astype(BF16)

    n_items = len(items)
    n_b = BS // RB
    b_done = 0
    for t in range(n_items + 2):
        if t < n_items:
            stage_a(t)
        if 0 <= t - 1 < n_items:
            stage_b(t - 1)
        if 0 <= t - 2 < n_items:
            stage_c(t - 2)
        want = min(n_b, ((t + 1) * n_b + n_items - 1) // n_items)
        while b_done < want:
            branch_b(b_done * RB)
            b_done += 1

    out = _nn(oc_ref[:, 0:D], woa_ref[...]) + _nn(oc_ref[:, D:2 * D], wobp_ref[...])
    out_ref[...] = out.astype(out_ref.dtype)


@jax.jit
def pallas_gated_mix__sliding_block__sliding_local_dilated__prompt_kernel(
    A_x: jax.Array,
    A_wqkv: jax.Array,
    A_wo: jax.Array,
    B_x: jax.Array,
    B_wqkv: jax.Array,
    B_wo: jax.Array,
    gate_w: jax.Array,
):
    xa = A_x.reshape(S, D)
    gw = gate_w.reshape(1, D)

    def const(shape):
        return pl.BlockSpec(shape, lambda i: (0, 0))

    rows = pl.BlockSpec((BS, D), lambda i: (i, 0))
    out = pl.pallas_call(
        _kernel,
        grid=(S // BS,),
        in_specs=[rows, const((D, 3 * D)), const((D, D)), const((D, 3 * D)), const((D, D)),
                  const((1, D))],
        out_specs=rows,
        out_shape=jax.ShapeDtypeStruct((S, D), A_x.dtype),
        scratch_shapes=[
            pltpu.VMEM((WIN + S, 768), BF16),
            pltpu.VMEM((NG * 48, WIN + S), BF16),
            pltpu.VMEM((D, 768), BF16),
            pltpu.VMEM((3 * D, D), BF16),
            pltpu.VMEM((D, D), BF16),
            pltpu.VMEM((NT, 3 * D, 128), F32),
            pltpu.VMEM((D, BS), F32),
            pltpu.VMEM((BS, D), F32),
            pltpu.VMEM((NT, PADB + S, 128), F32),
            pltpu.VMEM((NT, PADB + S, 128), F32),
            pltpu.VMEM((BS, 128), F32),
            pltpu.VMEM((BS, 2 * D), BF16),
            pltpu.VMEM((NS, 256, 384), F32),
            pltpu.VMEM((NP, 384, 384), BF16),
        ],
        compiler_params=pltpu.CompilerParams(
            dimension_semantics=("arbitrary",),
            vmem_limit_bytes=100 * 1024 * 1024),
    )(xa, A_wqkv, A_wo, B_wqkv, B_wo, gw)
    return out.reshape(1, S, D)
```

```python
import math

import jax
import jax.numpy as jnp
from jax import lax
import jax.experimental.pallas as pl
import jax.experimental.pallas.tpu as pltpu

S = 2048
D = 640
NT = D // 128
DH = 20
BS = 512
QB = 128
WIN = 256
NG = 16
PADB = 16
NS = 3
RB = 16
LOG2E = math.log2(math.e)
SCALE = DH ** -0.5
NEG = -1e9
BIGNEG = -(2.0 ** 30)

F32 = jnp.float32
BF16 = jnp.bfloat16


def _nn(a, b):
    return lax.dot_general(a, b, (((1,), (0,)), ((), ())), preferred_element_type=F32)


def _nt(a, b):
    return lax.dot_general(a, b, (((1,), (1,)), ((), ())), preferred_element_type=F32)


def _tt(a, b):
    return lax.dot_general(a, b, (((0,), (1,)), ((), ())), preferred_element_type=F32)


def _kernel(xa_ref, wa_hbm, woa_hbm, wb_hbm, wob_hbm, gw_ref, out_ref,
            kp_ref, vt_ref, wbt_ref, wobp_ref, tmp_ref,
            qt_ref, qb_ref, kb_ref, vb_ref, g_ref, oc_ref, s_ref,
            wa_ref, wb_ref, woa_ref, wob_ref, sems):
    i = pl.program_id(0)
    row0 = pl.multiple_of(i * BS, BS)

    def wcopy(k):
        if k < 3:
            c = (0, 2, 1)[k] * D
            return pltpu.make_async_copy(wa_hbm.at[:, c:c + D], wa_ref.at[:, c:c + D], sems.at[k])
        if k < 6:
            c = (1, 0, 2)[k - 3] * D
            return pltpu.make_async_copy(wb_hbm.at[:, c:c + D], wb_ref.at[:, c:c + D], sems.at[k])
        if k == 6:
            return pltpu.make_async_copy(wob_hbm, wob_ref, sems.at[k])
        return pltpu.make_async_copy(woa_hbm, woa_ref, sems.at[k])

    def prep_const():
        lane = lax.broadcasted_iota(jnp.int32, (WIN, 768), 1)
        kp_ref[0:WIN, :] = jnp.where(lane % 128 == 127, 1.0, 0.0).astype(BF16)
        vt_ref[:, 0:WIN] = jnp.zeros((NG * 48, WIN), BF16)
        kb_ref[:, 0:PADB, :] = jnp.zeros((NT, PADB, 128), F32)
        vb_ref[:, 0:PADB, :] = jnp.zeros((NT, PADB, 128), F32)

    def prep_wb(p):
        for n in range(NT):
            t_ = wb_ref[:, p * D + n * 128:p * D + (n + 1) * 128].T.astype(F32)
            for t in range(NT):
                tmp_ref[p, t, n * 128:(n + 1) * 128, :] = t_[:, t * 128:(t + 1) * 128]
        for t in range(NT):
            for d in range(DH):
                wbt_ref[p * D + d * 32:p * D + (d + 1) * 32, t * 128:(t + 1) * 128] = (
                    tmp_ref[p, t, pl.ds(d, 32, stride=DH), :].astype(BF16))

    def prep_wob():
        for t in range(NT):
            tmp_ref[3, t, :, :] = wob_ref[:, t * 128:(t + 1) * 128].astype(F32)
        for t in range(NT):
            for d in range(DH):
                wobp_ref[d * 32:(d + 1) * 32, t * 128:(t + 1) * 128] = (
                    tmp_ref[3, t, pl.ds(d, 32, stride=DH), :].astype(BF16))

    def gate():
        xa = xa_ref[...]
        gl = jnp.sum(xa.astype(F32) * gw_ref[...].astype(F32).reshape(1, D), axis=-1, keepdims=True)
        g_ref[...] = jnp.broadcast_to(jax.nn.sigmoid(gl), (BS, 128))

    def proj_q():
        qt_ref[...] = _tt(wa_ref[:, 0:D], xa_ref[...]) * (SCALE * LOG2E)

    def proj_v():
        vt = _tt(wa_ref[:, 2 * D:3 * D], xa_ref[...])
        ones8 = jnp.ones((8, BS), F32)
        for g in range(NG):
            blk = jnp.concatenate([vt[40 * g:40 * g + 40], ones8], axis=0).astype(BF16)
            vt_ref[48 * g:48 * g + 48, pl.ds(WIN + row0, BS)] = blk

    def proj_k():
        k = _nn(xa_ref[...], wa_ref[:, D:2 * D])
        lane = lax.broadcasted_iota(jnp.int32, (BS, 128), 1)
        tl = [k[:, t * 128:(t + 1) * 128] for t in range(NT)]
        for c in range(6):
            if c == 0:
                ch = tl[0]
            else:
                ch = pltpu.roll(tl[c - 1], 8 * c, 1)
                if c < NT:
                    ch = jnp.where(lane < 8 * c, ch, pltpu.roll(tl[c], 8 * c, 1))
            ch = jnp.where(lane < 127, ch, 0.0)
            kp_ref[pl.ds(WIN + row0, BS), c * 128:(c + 1) * 128] = ch.astype(BF16)

    def proj_b(p):
        r = _nt(xa_ref[...], wbt_ref[p * D:(p + 1) * D, :])
        if p == 0:
            qb_ref[...] = r * (SCALE * LOG2E)
        else:
            dst = kb_ref if p == 1 else vb_ref
            for t in range(NT):
                dst[t, pl.ds(PADB + row0, BS), :] = r[:, t * 128:(t + 1) * 128]

    r40 = lax.broadcasted_iota(jnp.int32, (40, 128), 0)
    l40 = lax.broadcasted_iota(jnp.int32, (40, 128), 1)
    m0 = (r40 < 20) & (l40 < 64)
    m1 = (r40 >= 20) & (l40 >= 64)
    h0row = r40 < 20
    lo64 = l40 < 64
    r8 = lax.broadcasted_iota(jnp.int32, (8, 128), 0)
    negrow = jnp.where(r8 == 7, BIGNEG, 0.0).astype(F32)

    def band_mask(nn):
        r64 = lax.broadcasted_iota(jnp.int32, (64, 128 * nn), 0)
        q64 = lax.broadcasted_iota(jnp.int32, (64, 128 * nn), 1) % 64
        return r64 > q64

    NB = BS // QB
    items = [(m, c, sub) for m in range(NB) for c in range(6) for sub in range(2)]
    mxs, outs, probs = {}, {}, {}

    def groups(c):
        return list(range(3 * c, min(3 * c + 3, NG)))

    def stage_a(n):
        m, c, sub = items[n]
        gs = groups(c)
        nn = len(gs)
        tiles = []
        for j, g in enumerate(gs):
            qt = qt_ref[40 * g:40 * g + 40, m * QB:(m + 1) * QB]
            rq = pltpu.roll(qt, 64, 1)
            if sub == 0:
                tq = jnp.where(m0, qt, jnp.where(m1, rq, 0.0))
            else:
                tq = jnp.where(m0, rq, jnp.where(m1, qt, 0.0))
            parts = []
            if j > 0:
                parts.append(jnp.zeros((40 * j, 128), F32))
            parts.append(tq)
            if j < 2:
                parts.append(jnp.zeros((80 - 40 * j, 128), F32))
            parts.append(negrow)
            tiles.append(jnp.concatenate(parts, axis=0))
        rhs = jnp.concatenate(tiles, axis=1).astype(BF16)
        kwin = kp_ref[pl.ds(row0 + m * QB + sub * 64, 320), c * 128:(c + 1) * 128]
        s = _nn(kwin, rhs)
        s = jnp.concatenate([jnp.where(band_mask(nn), s[0:64], s[256:320]), s[64:256]], axis=0)
        s_ref[n % NS, :, 0:128 * nn] = s
        mxs[n] = jnp.max(s, axis=0, keepdims=True)

    def stage_b(n):
        m, c, sub = items[n]
        nn = len(groups(c))
        p = jnp.exp2(s_ref[n % NS, :, 0:128 * nn] - mxs.pop(n))
        mk = band_mask(nn)
        ph = jnp.where(mk, p[0:64], 0.0)
        pt = jnp.where(mk, 0.0, p[0:64])
        z = jnp.zeros_like(ph)
        if sub == 0:
            ps = [jnp.concatenate([ph, p[64:128]], axis=0), p[128:256], jnp.concatenate([pt, z], axis=0)]
        else:
            ps = [jnp.concatenate([z, ph], axis=0), p[64:192], jnp.concatenate([p[192:256], pt], axis=0)]
        probs[n] = [[x[:, j * 128:(j + 1) * 128].astype(BF16) for j in range(nn)] for x in ps]

    def stage_c(n):
        m, c, sub = items[n]
        for j, g in enumerate(groups(c)):
            ot = sum(_nn(vt_ref[48 * g:48 * g + 48, pl.ds(row0 + (m + k) * QB, QB)], probs[n][k][j])
                     for k in range(3))
            outs[(g, sub)] = ot[0:40] * (1.0 / ot[40:41])
        if c == 5 and sub == 1:
            pieces = []
            for g in range(NG):
                o0, o1 = outs.pop((g, 0)), outs.pop((g, 1))
                a_ = jnp.where(h0row, o0, pltpu.roll(o0, 64, 1))
                b_ = jnp.where(h0row, pltpu.roll(o1, 64, 1), o1)
                pieces.append(jnp.where(lo64, a_, b_))
            oa = jnp.concatenate(pieces, axis=0).T
            gate = g_ref[m * QB:(m + 1) * QB, :]
            for t in range(NT):
                oc_ref[m * QB:(m + 1) * QB, t * 128:(t + 1) * 128] = (
                    oa[:, t * 128:(t + 1) * 128] * gate).astype(BF16)

    def branch_b(lr):
        q = [qb_ref[lr:lr + RB, t * 128:(t + 1) * 128] for t in range(NT)]
        logits = []
        for w in range(8):
            kr = PADB + row0 + lr - 2 * w
            acc = None
            for t in range(NT):
                pr = q[t] * kb_ref[t, pl.ds(kr, RB), :]
                acc = pr if acc is None else acc + pr
            acc = acc + pltpu.roll(acc, 64, 1)
            acc = acc + pltpu.roll(acc, 32, 1)
            if lr < 2 * w:
                pos = row0 + lr + lax.broadcasted_iota(jnp.int32, (RB, 128), 0)
                acc = jnp.where(pos >= 2 * w, acc, NEG)
            logits.append(acc)
        mx = logits[0]
        for w in range(1, 8):
            mx = jnp.maximum(mx, logits[w])
        es = [jnp.exp2(l - mx) for l in logits]
        den = es[0]
        for w in range(1, 8):
            den = den + es[w]
        fac = (1.0 - g_ref[lr:lr + RB, :]) / den
        for t in range(NT):
            acc = None
            for w in range(8):
                kr = PADB + row0 + lr - 2 * w
                pr = es[w] * vb_ref[t, pl.ds(kr, RB), :]
                acc = pr if acc is None else acc + pr
            oc_ref[lr:lr + RB, D + t * 128:D + (t + 1) * 128] = (acc * fac).astype(BF16)

    n_items = len(items)
    n_b = BS // RB
    @pl.when(i == 0)
    def _prep1():
        for k in (3, 4, 5, 0, 2, 1, 6, 7):
            wcopy(k).start()
        prep_const()
        for k, p_ in ((3, 1), (4, 0), (5, 2)):
            wcopy(k).wait()
            prep_wb(p_)
        for k in (0, 2, 1):
            wcopy(k).wait()
        wcopy(6).wait()
        prep_wob()
        wcopy(7).wait()

    gate()
    proj_b(1)
    proj_b(0)
    proj_b(2)

    for k, f in enumerate((proj_k, proj_q, proj_v)):
        f()
        for r in range(k * n_b // 3, (k + 1) * n_b // 3):
            branch_b(r * RB)

    for t in range(n_items + 2):
        if t < n_items:
            stage_a(t)
        if 0 <= t - 1 < n_items:
            stage_b(t - 1)
        if 0 <= t - 2 < n_items:
            stage_c(t - 2)

    out = _nn(oc_ref[:, 0:D], woa_ref[...]) + _nn(oc_ref[:, D:2 * D], wobp_ref[...])
    out_ref[...] = out.astype(out_ref.dtype)


@jax.jit
def pallas_gated_mix__sliding_block__sliding_local_dilated__prompt_kernel(
    A_x: jax.Array,
    A_wqkv: jax.Array,
    A_wo: jax.Array,
    B_x: jax.Array,
    B_wqkv: jax.Array,
    B_wo: jax.Array,
    gate_w: jax.Array,
):
    xa = A_x.reshape(S, D)
    gw = gate_w

    hbm = pl.BlockSpec(memory_space=pl.ANY)

    rows = pl.BlockSpec((BS, D), lambda i: (i, 0))
    out = pl.pallas_call(
        _kernel,
        grid=(S // BS,),
        in_specs=[rows, hbm, hbm, hbm, hbm, pl.BlockSpec((D,), lambda i: (0,))],
        out_specs=rows,
        out_shape=jax.ShapeDtypeStruct((S, D), A_x.dtype),
        scratch_shapes=[
            pltpu.VMEM((WIN + S, 768), BF16),
            pltpu.VMEM((NG * 48, WIN + S), BF16),
            pltpu.VMEM((3 * D, D), BF16),
            pltpu.VMEM((D, D), BF16),
            pltpu.VMEM((4, NT, D, 128), F32),
            pltpu.VMEM((D, BS), F32),
            pltpu.VMEM((BS, D), F32),
            pltpu.VMEM((NT, PADB + S, 128), F32),
            pltpu.VMEM((NT, PADB + S, 128), F32),
            pltpu.VMEM((BS, 128), F32),
            pltpu.VMEM((BS, 2 * D), BF16),
            pltpu.VMEM((NS, 256, 384), F32),
            pltpu.VMEM((D, 3 * D), BF16),
            pltpu.VMEM((D, 3 * D), BF16),
            pltpu.VMEM((D, D), BF16),
            pltpu.VMEM((D, D), BF16),
            pltpu.SemaphoreType.DMA((8,)),
        ],
        compiler_params=pltpu.CompilerParams(
            dimension_semantics=("arbitrary",),
            vmem_limit_bytes=100 * 1024 * 1024),
    )(xa, A_wqkv, A_wo, B_wqkv, B_wo, gw)
    return out.reshape(1, S, D)
```
